```python
import os as _os
_os.environ.setdefault("JAX_PLATFORMS", "cpu")
import jax
import jax.numpy as jnp

def _softmax(x, axis=-1):
    return jax.nn.softmax(x, axis=axis)
def _gelu(x):
    return jax.nn.gelu(x, approximate=True)
def _silu(x):
    return jax.nn.silu(x)
def _sigmoid(x):
    return jax.nn.sigmoid(x)
def _layernorm(x, axis=-1, eps=1e-5):
    m = jnp.mean(x, axis=axis, keepdims=True)
    v = jnp.var(x, axis=axis, keepdims=True)
    return (x - m) / jnp.sqrt(v + eps)
def _scatter_add(tgt, idx, src, axis=0):
    return tgt.at[idx].add(src)
def _segment_sum(src, seg, n):
    return jax.ops.segment_sum(src, seg, n)
class _Rng:
    def __init__(self, key):
        self._k = key
    def _next(self):
        self._k, sub = jax.random.split(self._k)
        return sub
    def normal(self, shape):
        return jax.random.normal(self._next(), shape, dtype=jnp.bfloat16)
    def randint(self, lo, hi, shape):
        return jax.random.randint(self._next(), shape, lo, hi, dtype=jnp.int32)
    def uniform(self, shape, lo=0.0, hi=1.0):
        return jax.random.uniform(self._next(), shape, jnp.bfloat16, lo, hi)
    def permutation(self, n):
        return jax.random.permutation(self._next(), n)


kernel_name = 'parallel_sum__ssm_conv_s5__glu_gated_swiglu__prompt'

def setup_inputs():
    _rng = _Rng(jax.random.key(int.from_bytes(__import__("os").urandom(4), "little")))
    _w = (lambda a: (lambda t: t.astype(jnp.bfloat16) if jnp.issubdtype(t.dtype, jnp.floating) else t)(jnp.asarray(a)))
    def _A_setup():
        B, S, D = 1, 2048, 640
        P = D
        Lambda_re = -0.5 * jnp.exp((lambda *s: _rng.normal(s) * 0.4)(P))
        Lambda_im = (lambda *s: _rng.normal(s) * 0.4)(P) * 1.0
        B_re = (lambda *s: _rng.normal(s) * 0.4)(P, D) * (D ** -0.5)
        B_im = (lambda *s: _rng.normal(s) * 0.4)(P, D) * (D ** -0.5)
        C_re = (lambda *s: _rng.normal(s) * 0.4)(D, P) * (P ** -0.5)
        C_im = (lambda *s: _rng.normal(s) * 0.4)(D, P) * (P ** -0.5)
        log_dt = (lambda *s: _rng.normal(s) * 0.4)(P) * 0.3 - 2.0
        Dskip = (lambda *s: _rng.normal(s) * 0.4)(D)
        return {
            "x": _w((lambda *s: _rng.normal(s) * 0.05)(B, S, D)),
            "Lambda_re": _w(Lambda_re),
            "Lambda_im": _w(Lambda_im),
            "B_re": _w(B_re),
            "B_im": _w(B_im),
            "C_re": _w(C_re),
            "C_im": _w(C_im),
            "log_dt": _w(log_dt),
            "Dskip": _w(Dskip),
        }
    _A_in = _A_setup()

    def _B_setup():
        B, S, D, F = 1, 2048, 640, 1728
        return {
            "x": _w((lambda *s: _rng.normal(s) * 0.05)(B, S, D)),
            "w1": _w((lambda *s: _rng.normal(s) * 0.1)(D, F) * (2.0 / D) ** 0.5),
            "w3": _w((lambda *s: _rng.normal(s) * 0.1)(D, F) * (2.0 / D) ** 0.5),
            "w2": _w((lambda *s: _rng.normal(s) * 0.1)(F, D) * (2.0 / F) ** 0.5),
        }
    _B_in = _B_setup()

    return {
        "A_x": _A_in["x"],
        "A_Lambda_re": _A_in["Lambda_re"],
        "A_Lambda_im": _A_in["Lambda_im"],
        "A_B_re": _A_in["B_re"],
        "A_B_im": _A_in["B_im"],
        "A_C_re": _A_in["C_re"],
        "A_C_im": _A_in["C_im"],
        "A_log_dt": _A_in["log_dt"],
        "A_Dskip": _A_in["Dskip"],
        "B_x": _B_in["x"],
        "B_w1": _B_in["w1"],
        "B_w3": _B_in["w3"],
        "B_w2": _B_in["w2"],
    }

def reference(A_x, A_Lambda_re, A_Lambda_im, A_B_re, A_B_im, A_C_re, A_C_im, A_log_dt, A_Dskip, B_x, B_w1, B_w3, B_w2):
    def _A_ref(x, Lambda_re, Lambda_im, B_re, B_im, C_re, C_im, log_dt, Dskip):
        Bsz, L, H = x.shape
        Lam = Lambda_re + 1j * Lambda_im
        Bmat = B_re + 1j * B_im
        Cmat = C_re + 1j * C_im
        dt = jnp.exp(log_dt)
        Lam_bar = jnp.exp(dt * Lam)
        B_bar = ((Lam_bar - 1.0) / Lam)[:, None] * Bmat
        Bu = jnp.einsum("bld,pd->blp", x + 0j, B_bar)
        h = jnp.zeros_like(Bu[:, 0, :])
        hs = []
        for t in range(L):
            h = Lam_bar[None, :] * h + Bu[:, t, :]
            hs.append(h)
        hseq = jnp.stack(hs, 1)
        y = 2.0 * jnp.einsum("blp,dp->bld", hseq, Cmat).real + x * Dskip[None, None, :]
        return y

    def _B_ref(x, w1, w3, w2):
        gate = jnp.einsum("bsd,df->bsf", x, w1)
        up = jnp.einsum("bsd,df->bsf", x, w3)
        h = _silu(gate) * up
        out = jnp.einsum("bsf,fd->bsd", h, w2)
        return out

    x = A_x
    xn = _layernorm(x, axis=-1)
    return x + _A_ref(xn, A_Lambda_re, A_Lambda_im, A_B_re, A_B_im, A_C_re, A_C_im, A_log_dt, A_Dskip) + _B_ref(xn, B_w1, B_w3, B_w2)
```

```python
import jax
import jax.numpy as jnp
from jax import lax
import jax.experimental.pallas as pl
import jax.experimental.pallas.tpu as pltpu

T = 512
L = T // 8
S, D, F = 2048, 640, 1728
NB = S // T
NP = D // 128
FM = (F // 128) * 128
FT = F - FM
NF = FM // 128
NS = 4
f_, b_ = (lambda j: ('f', j)), (lambda j: ('b', j))
REGIONS = [[f_(0), f_(1)], [b_(0), f_(2)], [b_(1), f_(3), b_(2), f_(4)],
           [b_(3), f_(5), f_(6), b_(4), f_(7), f_(8)], [f_(9), f_(10), f_(11), f_(12)]]
f32 = jnp.float32
bf16 = jnp.bfloat16
NT = (((1,), (1,)), ((), ()))


def cmul(ar, ai, br, bi):
    return ar * br - ai * bi, ar * bi + ai * br


def nt(a, b):
    return lax.dot_general(a, b, NT, preferred_element_type=f32)


def kern(x_hbm, lre_hbm, lim_hbm, ldt_hbm, dsk_hbm, bre_hbm, bim_hbm, cre_hbm, cim_hbm, w1_hbm, w3_hbm, w2_hbm,
         o_hbm, xv, vec, bre, bim, cre, cim, w1, w3, wt, w2, c2r, c2i, xf, ov, xbv, basev, hrv, hiv, sem):
    n = [0]
    def cp(src, dst, go=True):
        c = pltpu.make_async_copy(src, dst, sem.at[n[0]]); n[0] += 1
        if go:
            c.start()
        return c
    rows = lambda r, a, b: r.at[pl.ds(a, b - a)]
    first = [cp(rows(x_hbm, 0, T), rows(xv, 0, T))]
    first += [cp(h, vec[k]) for k, h in enumerate((lre_hbm, lim_hbm, ldt_hbm, dsk_hbm))]
    regions = REGIONS
    dp = lambda a, b: cp(a, b, False)
    dw = []
    for k, reg in enumerate(regions):
        cs = []
        for kind, srcs in (('b', ((bre_hbm, bre), (bim_hbm, bim))), ('f', ((w1_hbm, w1), (w3_hbm, w3)))):
            js = [j for kd, j in reg if kd == kind]
            if js:
                cs += [dp(rows(h, js[0] * 128, js[-1] * 128 + 128), rows(v, js[0] * 128, js[-1] * 128 + 128)) for h, v in srcs]
        dw.append(cs)
    dlast = [dp(rows(w1_hbm, FM, F), rows(wt, 0, FT)), dp(rows(w3_hbm, FM, F), rows(wt, FT, 2 * FT)),
             dp(cre_hbm, cre), dp(cim_hbm, cim), dp(rows(x_hbm, T, 2 * T), rows(xv, T, 2 * T))]
    dw[-1].append(dp(w2_hbm, w2))
    dxr = dp(rows(x_hbm, 2 * T, S), rows(xv, 2 * T, S))
    dw.append(dlast)
    for c in first[1:]:
        c.wait()
    rd = lambda k: vec[k][...].astype(f32).reshape(1, D)
    dsk = jnp.broadcast_to(rd(3), (16, D))
    LP = L + 4

    def ln_tasks(b):
        rs = {}
        def conv(q):
            for c in range(NP):
                xf[c, q * LP:q * LP + L] = xv[b * T + q * L:b * T + (q + 1) * L, c * 128:(c + 1) * 128].astype(f32)
        def norm(r):
            x = jnp.concatenate([jnp.concatenate(
                [xf[c, pl.ds(t, 8, stride=LP), :] for c in range(NP)], axis=1) for t in (2 * r, 2 * r + 1)], axis=0)
            w = 16 if b == 0 else 1
            xc = x - jnp.sum(x, axis=-1, keepdims=True) * (jnp.where(rs[r - w] < 0.0, 0.0, 1.0 / D) if r >= w else 1.0 / D)
            rs[r] = lax.rsqrt(jnp.mean(xc * xc, axis=-1, keepdims=True) + 1e-5)
            xn = xc * rs[r]
            xbv[b, 16 * r:16 * r + 16] = xn.astype(bf16)
            basev[b, 16 * r:16 * r + 16] = x + xn * dsk
        return [lambda q=q: conv(q) for q in range(8)] + [lambda r=r: norm(r) for r in range(T // 16)]

    prm = {}

    def params():
        lre, lim, dt = rd(0), rd(1), jnp.exp(rd(2))
        mag = jnp.exp(dt * lre)
        ar = mag * jnp.cos(dt * lim); ai = mag * jnp.sin(dt * lim)
        den = lre * lre + lim * lim
        prm['c'] = (2.0 * ((ar - 1.0) * lre + ai * lim) / den, 2.0 * (ai * lre - (ar - 1.0) * lim) / den)
        pr = jnp.broadcast_to(ar, (8, D)); pi = jnp.broadcast_to(ai, (8, D))
        prm['a'] = (pr, pi)
        row = lax.broadcasted_iota(jnp.int32, (8, D), 0)
        for _ in range(L.bit_length() - 1):
            pr, pi = cmul(pr, pi, pr, pi)
        for k in range(3):
            prm[k] = (jnp.where(row >= (1 << k), pr, 0.0), jnp.where(row >= (1 << k), pi, 0.0))
            if k < 2:
                pr, pi = cmul(pr, pi, pr, pi)

    def cprep(r):
        sl = slice(16 * r, 16 * r + 16)
        tr, ti = cmul(cre[sl].astype(f32), cim[sl].astype(f32), *prm['c'])
        c2r[sl] = tr.astype(bf16); c2i[sl] = (-ti).astype(bf16)

    carry = [None] * NP

    def scan_tasks(b, p, ur, ui):
        sl = slice(p * 128, p * 128 + 128)
        st = {}
        def step(z, t):
            a_r, a_i = prm['a'][0][:, sl], prm['a'][1][:, sl]
            return ((a_r * z[0] + ur[8 * t:8 * t + 8]) - a_i * z[1], (a_r * z[1] + ui[8 * t:8 * t + 8]) + a_i * z[0])
        def p1(t0):
            for t in range(t0, t0 + 8):
                st['z'] = step(st['z'], t) if t else (ur[0:8], ui[0:8])
        def mid():
            row0 = lax.broadcasted_iota(jnp.int32, (8, 128), 0) == 0
            z = [jnp.where(row0, carry[p][q] if b else 0.0, pltpu.roll(st['z'][q], 1, 0)) for q in range(2)]
            for q in range(3):
                tr, ti = cmul(prm[q][0][:, sl], prm[q][1][:, sl], pltpu.roll(z[0], 1 << q, 0), pltpu.roll(z[1], 1 << q, 0))
                z = [z[0] + tr, z[1] + ti]
            st['z'] = z
        def p2(t0):
            for t in range(t0, t0 + 8, 2):
                z0 = step(st['z'], t); z1 = step(z0, t + 1); st['z'] = z1
                hrv[b % 2, 8 * t:8 * t + 16, sl] = jnp.concatenate([z0[0], z1[0]], 0).astype(bf16)
                hiv[b % 2, 8 * t:8 * t + 16, sl] = jnp.concatenate([z0[1], z1[1]], 0).astype(bf16)
            if t0 + 8 == L:
                carry[p] = (pltpu.roll(z1[0], 1, 0), pltpu.roll(z1[1], 1, 0))
        return [lambda t=t: p1(t) for t in range(0, L, 8)] + [mid] + [lambda t=t: p2(t) for t in range(0, L, 8)]

    params()
    first[0].wait()
    for c in dw[0]:
        c.start()
    for t_ in ln_tasks(0):
        t_()
    queue = []

    def side(k):
        for _ in range(min(k, len(queue))):
            queue.pop(0)()

    douts = []
    ov4 = ov.reshape(NB, NP, 8, L + 8, 128)
    for b in range(NB):
        hh = []
        for k, reg in enumerate(regions):
            if b == 0:
                for c in dw[k]:
                    c.wait()
                for c in dw[k + 1]:
                    c.start()
            elif k == 4:
                if b == 1:
                    dxr.wait()
                douts += [cp(ov4.at[b - 1, c, :, pl.ds(0, L)], o_hbm.at[pl.ds(b * 8 - 8, 8), :, pl.ds(c * 128, 128)]) for c in range(NP)]
            for kind, j in reg:
                sl = slice(j * 128, j * 128 + 128)
                ns = NS
                u0 = nt(xbv[b], (bre if kind == 'b' else w1)[sl]); side(ns)
                u1 = nt(xbv[b], (bim if kind == 'b' else w3)[sl])
                if kind == 'b':
                    queue.extend(scan_tasks(b, j, u0, u1))
                else:
                    g = 0.5 * u0
                    hh.append(((g + g * jnp.tanh(g)) * u1).astype(bf16))
                side(ns)
        if b == 0:
            for c in dlast:
                c.wait()
            dxr.start()
        gu = nt(xbv[b], wt[...])
        g = 0.5 * gu
        ht = ((g + g * jnp.tanh(g)) * pltpu.roll(gu, FT, 1)).astype(bf16)[:, :FT]
        side(len(queue))
        hh = jnp.concatenate(hh, 1)
        if b + 1 < NB:
            queue.extend(ln_tasks(b + 1))
        for c in range(NP):
            sl = slice(c * 128, c * 128 + 128)
            acc = basev[b, :, sl] + jnp.dot(hh[:, :640], w2[:640, sl], preferred_element_type=f32); side(2)
            if b == 0:
                for r in range(8 * c, 8 * c + 8):
                    cprep(r)
            acc = acc + jnp.dot(hh[:, 640:], w2[640:FM, sl], preferred_element_type=f32); side(3)
            acc = acc + jnp.dot(ht, w2[FM:, sl], preferred_element_type=f32)
            acc = acc + nt(hrv[b % 2], c2r[sl]); side(2)
            acc = acc + nt(hiv[b % 2], c2i[sl]); side(2)
            for t in range(L):
                ov[b, c, pl.ds(t, 8, stride=L + 8), :] = acc[8 * t:8 * t + 8]
            if b == NB - 1 and c in (3, 4):
                douts += [cp(ov4.at[b, e, :, pl.ds(0, L)], o_hbm.at[pl.ds(b * 8, 8), :, pl.ds(e * 128, 128)]) for e in (range(4) if c == 3 else (4,))]
    for c in douts:
        c.wait()


@jax.jit
def pallas_parallel_sum__ssm_conv_s5__glu_gated_swiglu__prompt_kernel(
        A_x, A_Lambda_re, A_Lambda_im, A_B_re, A_B_im, A_C_re, A_C_im, A_log_dt, A_Dskip, B_x, B_w1, B_w3, B_w2):
    args = (A_x.reshape(S, D), A_Lambda_re, A_Lambda_im, A_log_dt, A_Dskip,
            A_B_re, A_B_im, A_C_re, A_C_im, B_w1.T, B_w3.T, B_w2)
    V = pltpu.VMEM
    out = pl.pallas_call(
        kern,
        in_specs=[pl.BlockSpec(memory_space=pltpu.HBM)] * len(args),
        out_specs=pl.BlockSpec(memory_space=pltpu.HBM),
        out_shape=jax.ShapeDtypeStruct((S // L, L, D), f32),
        scratch_shapes=[V((S, D), bf16), [V((D,), bf16) for _ in range(4)]] + [V((D, D), bf16)] * 4 + [V((FM, D), bf16)] * 2
        + [V((2 * FT, D), bf16), V((F, D), bf16), V((D, D), bf16), V((D, D), bf16), V((NP, T + 32, 128), f32),
           V((NB, NP, T + 64, 128), f32), V((NB, T, D), bf16), V((NB, T, D), f32), V((2, T, D), bf16), V((2, T, D), bf16), pltpu.SemaphoreType.DMA((64,))],
        compiler_params=pltpu.CompilerParams(vmem_limit_bytes=100 * 2**20),
    )(*args)
    return out.reshape(1, S, D)
```

```python
import jax
import jax.numpy as jnp
from jax import lax
import jax.experimental.pallas as pl
import jax.experimental.pallas.tpu as pltpu

T = 512
L = T // 8
S, D, F = 2048, 640, 1728
NB = S // T
NP = D // 128
FM = (F // 128) * 128
FT = F - FM
NF = FM // 128
NS = 4
f_, b_ = (lambda j: ('f', j)), (lambda j: ('b', j))
REGIONS = [[f_(0), f_(1)], [b_(0), f_(2)], [b_(1), f_(3), b_(2), f_(4)],
           [b_(3), f_(5), f_(6), b_(4), f_(7), f_(8)], [f_(9), f_(10), f_(11), f_(12)]]
f32 = jnp.float32
bf16 = jnp.bfloat16
NT = (((1,), (1,)), ((), ()))


def cmul(ar, ai, br, bi):
    return ar * br - ai * bi, ar * bi + ai * br


def nt(a, b):
    return lax.dot_general(a, b, NT, preferred_element_type=f32)


def kern(x_hbm, lre_hbm, lim_hbm, ldt_hbm, dsk_hbm, bre_hbm, bim_hbm, cre_hbm, cim_hbm, w1_hbm, w3_hbm, w2_hbm,
         o_hbm, xv, vec, bre, bim, cre, cim, w1, w3, wt, w2, c2r, c2i, xf, ov, xbv, basev, hrv, hiv, sem):
    n = [0]
    def cp(src, dst, go=True):
        c = pltpu.make_async_copy(src, dst, sem.at[n[0]]); n[0] += 1
        if go:
            c.start()
        return c
    rows = lambda r, a, b: r.at[pl.ds(a, b - a)]
    first = [cp(rows(x_hbm, 0, T), rows(xv, 0, T))]
    first += [cp(h, vec[k]) for k, h in enumerate((lre_hbm, lim_hbm, ldt_hbm, dsk_hbm))]
    regions = REGIONS
    dp = lambda a, b: cp(a, b, False)
    dw = []
    for k, reg in enumerate(regions):
        cs = []
        for kind, srcs in (('b', ((bre_hbm, bre), (bim_hbm, bim))), ('f', ((w1_hbm, w1), (w3_hbm, w3)))):
            js = [j for kd, j in reg if kd == kind]
            if js:
                cs += [dp(rows(h, js[0] * 128, js[-1] * 128 + 128), rows(v, js[0] * 128, js[-1] * 128 + 128)) for h, v in srcs]
        dw.append(cs)
    dlast = [dp(rows(w1_hbm, FM, F), rows(wt, 0, FT)), dp(rows(w3_hbm, FM, F), rows(wt, FT, 2 * FT)),
             dp(cre_hbm, cre), dp(cim_hbm, cim), dp(rows(x_hbm, T, S), rows(xv, T, S))]
    dw[-1].append(dp(w2_hbm, w2))
    dw.append(dlast)
    for c in first[1:]:
        c.wait()
    rd = lambda k: vec[k][...].astype(f32).reshape(1, D)
    dsk = jnp.broadcast_to(rd(3), (16, D))
    LP = L + 4

    def ln_tasks(b):
        rs = {}
        def conv(q):
            for c in range(NP):
                xf[c, q * LP:q * LP + L] = xv[b * T + q * L:b * T + (q + 1) * L, c * 128:(c + 1) * 128].astype(f32)
        def norm(r):
            x = jnp.concatenate([jnp.concatenate(
                [xf[c, pl.ds(t, 8, stride=LP), :] for c in range(NP)], axis=1) for t in (2 * r, 2 * r + 1)], axis=0)
            w = 16 if b == 0 else 1
            xc = x - jnp.sum(x, axis=-1, keepdims=True) * (jnp.where(rs[r - w] < 0.0, 0.0, 1.0 / D) if r >= w else 1.0 / D)
            rs[r] = lax.rsqrt(jnp.mean(xc * xc, axis=-1, keepdims=True) + 1e-5)
            xn = xc * rs[r]
            xbv[b, 16 * r:16 * r + 16] = xn.astype(bf16)
            basev[b, 16 * r:16 * r + 16] = x + xn * dsk
        return [lambda q=q: conv(q) for q in range(8)] + [lambda r=r: norm(r) for r in range(T // 16)]

    prm = {}

    def params():
        lre, lim, dt = rd(0), rd(1), jnp.exp(rd(2))
        mag = jnp.exp(dt * lre)
        ar = mag * jnp.cos(dt * lim); ai = mag * jnp.sin(dt * lim)
        den = lre * lre + lim * lim
        prm['c'] = (2.0 * ((ar - 1.0) * lre + ai * lim) / den, 2.0 * (ai * lre - (ar - 1.0) * lim) / den)
        pr = jnp.broadcast_to(ar, (8, D)); pi = jnp.broadcast_to(ai, (8, D))
        prm['a'] = (pr, pi)
        row = lax.broadcasted_iota(jnp.int32, (8, D), 0)
        for _ in range(L.bit_length() - 1):
            pr, pi = cmul(pr, pi, pr, pi)
        for k in range(3):
            prm[k] = (jnp.where(row >= (1 << k), pr, 0.0), jnp.where(row >= (1 << k), pi, 0.0))
            if k < 2:
                pr, pi = cmul(pr, pi, pr, pi)

    def cprep(r):
        sl = slice(16 * r, 16 * r + 16)
        tr, ti = cmul(cre[sl].astype(f32), cim[sl].astype(f32), *prm['c'])
        c2r[sl] = tr.astype(bf16); c2i[sl] = (-ti).astype(bf16)

    carry = [None] * NP

    def scan_tasks(b, p, ur, ui):
        sl = slice(p * 128, p * 128 + 128)
        st = {}
        def step(z, t):
            a_r, a_i = prm['a'][0][:, sl], prm['a'][1][:, sl]
            return ((a_r * z[0] + ur[8 * t:8 * t + 8]) - a_i * z[1], (a_r * z[1] + ui[8 * t:8 * t + 8]) + a_i * z[0])
        def p1(t0):
            for t in range(t0, t0 + 8):
                st['z'] = step(st['z'], t) if t else (ur[0:8], ui[0:8])
        def mid():
            row0 = lax.broadcasted_iota(jnp.int32, (8, 128), 0) == 0
            z = [jnp.where(row0, carry[p][q] if b else 0.0, pltpu.roll(st['z'][q], 1, 0)) for q in range(2)]
            for q in range(3):
                tr, ti = cmul(prm[q][0][:, sl], prm[q][1][:, sl], pltpu.roll(z[0], 1 << q, 0), pltpu.roll(z[1], 1 << q, 0))
                z = [z[0] + tr, z[1] + ti]
            st['z'] = z
        def p2(t0):
            for t in range(t0, t0 + 8, 2):
                z0 = step(st['z'], t); z1 = step(z0, t + 1); st['z'] = z1
                hrv[b % 2, 8 * t:8 * t + 16, sl] = jnp.concatenate([z0[0], z1[0]], 0).astype(bf16)
                hiv[b % 2, 8 * t:8 * t + 16, sl] = jnp.concatenate([z0[1], z1[1]], 0).astype(bf16)
            if t0 + 8 == L:
                carry[p] = (pltpu.roll(z1[0], 1, 0), pltpu.roll(z1[1], 1, 0))
        return [lambda t=t: p1(t) for t in range(0, L, 8)] + [mid] + [lambda t=t: p2(t) for t in range(0, L, 8)]

    for c in dw[0]:
        c.start()
    params()
    first[0].wait()
    for c in dw[1]:
        c.start()
    for t_ in ln_tasks(0):
        t_()
    queue = []

    def side(k):
        for _ in range(min(k, len(queue))):
            queue.pop(0)()

    douts = []
    ov4 = ov.reshape(NB, NP, 8, L + 8, 128)
    for b in range(NB):
        hh = []
        for k, reg in enumerate(regions):
            if b == 0:
                for c in dw[k]:
                    c.wait()
                for c in (dw[k + 2] if k + 2 < len(dw) else []):
                    c.start()
            elif k == 1:
                douts += [cp(ov4.at[b - 1, c, :, pl.ds(0, L)], o_hbm.at[pl.ds(b * 8 - 8, 8), :, pl.ds(c * 128, 128)]) for c in range(NP)]
            for kind, j in reg:
                sl = slice(j * 128, j * 128 + 128)
                ns = NS
                u0 = nt(xbv[b], (bre if kind == 'b' else w1)[sl]); side(ns)
                u1 = nt(xbv[b], (bim if kind == 'b' else w3)[sl])
                if kind == 'b':
                    queue.extend(scan_tasks(b, j, u0, u1))
                else:
                    g = 0.5 * u0
                    hh.append(((g + g * jnp.tanh(g)) * u1).astype(bf16))
                side(ns)
        if b == 0:
            for c in dlast:
                c.wait()
        gu = nt(xbv[b], wt[...])
        g = 0.5 * gu
        ht = ((g + g * jnp.tanh(g)) * pltpu.roll(gu, FT, 1)).astype(bf16)[:, :FT]
        side(len(queue))
        hh = jnp.concatenate(hh, 1)
        if b + 1 < NB:
            queue.extend(ln_tasks(b + 1))
        for c in range(NP):
            sl = slice(c * 128, c * 128 + 128)
            acc = basev[b, :, sl] + jnp.dot(hh[:, :640], w2[:640, sl], preferred_element_type=f32); side(2)
            if b == 0:
                for r in range(8 * c, 8 * c + 8):
                    cprep(r)
            acc = acc + jnp.dot(hh[:, 640:], w2[640:FM, sl], preferred_element_type=f32); side(3)
            acc = acc + jnp.dot(ht, w2[FM:, sl], preferred_element_type=f32)
            acc = acc + nt(hrv[b % 2], c2r[sl]); side(2)
            acc = acc + nt(hiv[b % 2], c2i[sl]); side(2)
            for t in range(L):
                ov[b, c, pl.ds(t, 8, stride=L + 8), :] = acc[8 * t:8 * t + 8]
            if b == NB - 1 and c in (3, 4):
                douts += [cp(ov4.at[b, e, :, pl.ds(0, L)], o_hbm.at[pl.ds(b * 8, 8), :, pl.ds(e * 128, 128)]) for e in (range(4) if c == 3 else (4,))]
    for c in douts:
        c.wait()


@jax.jit
def pallas_parallel_sum__ssm_conv_s5__glu_gated_swiglu__prompt_kernel(
        A_x, A_Lambda_re, A_Lambda_im, A_B_re, A_B_im, A_C_re, A_C_im, A_log_dt, A_Dskip, B_x, B_w1, B_w3, B_w2):
    args = (A_x.reshape(S, D), A_Lambda_re, A_Lambda_im, A_log_dt, A_Dskip,
            A_B_re, A_B_im, A_C_re, A_C_im, B_w1.T, B_w3.T, B_w2)
    V = pltpu.VMEM
    out = pl.pallas_call(
        kern,
        in_specs=[pl.BlockSpec(memory_space=pltpu.HBM)] * len(args),
        out_specs=pl.BlockSpec(memory_space=pltpu.HBM),
        out_shape=jax.ShapeDtypeStruct((S // L, L, D), f32),
        scratch_shapes=[V((S, D), bf16), [V((D,), bf16) for _ in range(4)]] + [V((D, D), bf16)] * 4 + [V((FM, D), bf16)] * 2
        + [V((2 * FT, D), bf16), V((F, D), bf16), V((D, D), bf16), V((D, D), bf16), V((NP, T + 32, 128), f32),
           V((NB, NP, T + 64, 128), f32), V((NB, T, D), bf16), V((NB, T, D), f32), V((2, T, D), bf16), V((2, T, D), bf16), pltpu.SemaphoreType.DMA((64,))],
        compiler_params=pltpu.CompilerParams(vmem_limit_bytes=100 * 2**20),
    )(*args)
    return out.reshape(1, S, D)
```
